```python
import os as _os
_os.environ.setdefault("JAX_PLATFORMS", "cpu")
import jax
import jax.numpy as jnp

def _softmax(x, axis=-1):
    return jax.nn.softmax(x, axis=axis)
def _gelu(x):
    return jax.nn.gelu(x, approximate=True)
def _silu(x):
    return jax.nn.silu(x)
def _sigmoid(x):
    return jax.nn.sigmoid(x)
def _layernorm(x, axis=-1, eps=1e-5):
    m = jnp.mean(x, axis=axis, keepdims=True)
    v = jnp.var(x, axis=axis, keepdims=True)
    return (x - m) / jnp.sqrt(v + eps)
def _scatter_add(tgt, idx, src, axis=0):
    return tgt.at[idx].add(src)
def _segment_sum(src, seg, n):
    return jax.ops.segment_sum(src, seg, n)
class _Rng:
    def __init__(self, key):
        self._k = key
    def _next(self):
        self._k, sub = jax.random.split(self._k)
        return sub
    def normal(self, shape):
        return jax.random.normal(self._next(), shape, dtype=jnp.bfloat16)
    def randint(self, lo, hi, shape):
        return jax.random.randint(self._next(), shape, lo, hi, dtype=jnp.int32)
    def uniform(self, shape, lo=0.0, hi=1.0):
        return jax.random.uniform(self._next(), shape, jnp.bfloat16, lo, hi)
    def permutation(self, n):
        return jax.random.permutation(self._next(), n)


kernel_name = 'sequential_preLN__mha_block__dense_activation_mish__prompt'

def setup_inputs():
    _rng = _Rng(jax.random.key(int.from_bytes(__import__("os").urandom(4), "little")))
    _w = (lambda a: (lambda t: t.astype(jnp.bfloat16) if jnp.issubdtype(t.dtype, jnp.floating) else t)(jnp.asarray(a)))
    def _A_setup():
        B, S, D, H = 1, 2048, 576, 32
        return {
            "x": _w((lambda *s: _rng.normal(s) * 0.05)(B, S, D)),
            "wqkv": _w((lambda *s: _rng.normal(s) * 0.05)(D, 3 * D)),
            "wo": _w((lambda *s: _rng.normal(s) * 0.05)(D, D)),
        }
    _A_in = _A_setup()

    def _B_setup():
        B, S, D, F = 1, 2048, 576, 4608
        return {
            "x": _w((lambda *s: _rng.normal(s) * 0.05)(B, S, D)),
            "w1": _w((lambda *s: _rng.normal(s) * 1.6)(D, F) * (D ** -0.5)),
            "b1": _w((lambda *s: _rng.normal(s) * 0.05)(F)),
            "w2": _w((lambda *s: _rng.normal(s) * 0.05)(F, D) * (F ** -0.5)),
        }
    _B_in = _B_setup()

    return {
        "A_x": _A_in["x"],
        "A_wqkv": _A_in["wqkv"],
        "A_wo": _A_in["wo"],
        "B_x": _B_in["x"],
        "B_w1": _B_in["w1"],
        "B_b1": _B_in["b1"],
        "B_w2": _B_in["w2"],
    }

def reference(A_x, A_wqkv, A_wo, B_x, B_w1, B_b1, B_w2):
    def _A_ref(x, wqkv, wo):
        B, S, D = x.shape
        H = 32
        Dh = D // H
        qkv = (lambda x, *d: x.transpose(*d))((x @ wqkv).reshape(B, S, 3, H, Dh), 2, 0, 3, 1, 4)
        q, k, v = qkv[0], qkv[1], qkv[2]
        scores = jnp.einsum("bhqd,bhkd->bhqk", q, k) * (Dh ** -0.5)
        p = _softmax(scores, axis=-1)
        o = jnp.einsum("bhqk,bhkd->bhqd", p, v)
        return (lambda x, *d: x.transpose(*d))(o, 0, 2, 1, 3).reshape(B, S, D) @ wo

    def _B_ref(x, w1, b1, w2):
        h = jnp.einsum("bsd,df->bsf", x, w1) + b1
        sp = jnp.log1p(jnp.exp(-jnp.abs(h))) + jnp.where(h > 0, h, jnp.zeros_like(h))
        act = h * jnp.tanh(sp)
        return jnp.einsum("bsf,fd->bsd", act, w2)

    x = A_x
    h = x + _A_ref(_layernorm(x, axis=-1), A_wqkv, A_wo)
    h2 = h + _B_ref(_layernorm(h, axis=-1), B_w1, B_b1, B_w2)
    return h2
```

```python
import functools
import math

import jax
import jax.numpy as jnp
import jax.experimental.pallas as pl
import jax.experimental.pallas.tpu as pltpu

_H = 32
_LANES = 128
_WIN = 32
_EPS = 1e-5
_LOG2E = math.log2(math.e)


def _layernorm(x):
    m = jnp.mean(x, axis=-1, keepdims=True)
    xc = x - m
    v = jnp.mean(xc * xc, axis=-1, keepdims=True)
    return xc * jax.lax.rsqrt(v + _EPS)


def _kernel(x_ref, wk_ref, wqv_ref, wo_ref, w1_ref, b1_ref, w2_ref, o_ref,
            k_sc, qt_sc, vt_sc, ot_sc, st_a, st_b, m_a, m_b,
            *, S, D, Dh, hpg, ngrp, tq, fchunk):
    step = pl.program_id(0)
    G = ngrp * _LANES

    @pl.when(step == 0)
    def _prologue():
        xn = _layernorm(x_ref[...].astype(jnp.float32)).astype(jnp.bfloat16)
        k = jnp.dot(xn, wk_ref[...], preferred_element_type=jnp.float32)
        for g in range(ngrp):
            k_sc[g] = k[:, g * _LANES:(g + 1) * _LANES].astype(jnp.bfloat16)
        qv = jnp.dot(xn, wqv_ref[...], preferred_element_type=jnp.float32)
        qscale = (Dh ** -0.5) * _LOG2E
        for g in range(ngrp):
            qt_sc[g] = (qv[:, g * _LANES:(g + 1) * _LANES] * qscale).T.astype(jnp.bfloat16)
            vt_sc[g] = qv[:, G + g * _LANES:G + (g + 1) * _LANES].T.astype(jnp.bfloat16)

    q0 = pl.multiple_of(step * tq, tq)
    row_q = jax.lax.broadcasted_iota(jnp.int32, (_LANES, tq), 0)
    row_v = jax.lax.broadcasted_iota(jnp.int32, (_WIN, S), 0)
    row_o = jax.lax.broadcasted_iota(jnp.int32, (_WIN, tq), 0)

    def scores(h, st_sc, m_sc):
        g = h // hpg
        lo = (h % hpg) * Dh
        qt_g = qt_sc[g, :, pl.ds(q0, tq)]
        in_head = jnp.logical_and(row_q >= lo, row_q < lo + Dh)
        qt_h = jnp.where(in_head, qt_g, jnp.zeros_like(qt_g))
        st = jnp.dot(k_sc[g], qt_h, preferred_element_type=jnp.float32)
        st_sc[...] = st
        m_sc[...] = jnp.max(st, axis=0, keepdims=True)

    def values(h, st_sc, m_sc):
        g = h // hpg
        lo = (h % hpg) * Dh
        w0 = pl.multiple_of((lo // 16) * 16, 16)
        off = lo - w0
        pt = jnp.exp2(st_sc[...] - m_sc[...]).astype(jnp.bfloat16)
        vwin = vt_sc[g, pl.ds(w0, _WIN), :]
        v_in = jnp.logical_and(row_v >= off, row_v < off + Dh)
        lhs = jnp.where(v_in, vwin, jnp.ones_like(vwin))
        ot = jnp.dot(lhs, pt, preferred_element_type=jnp.float32)
        l = ot[_WIN - 1:_WIN, :]
        o_in = jnp.logical_and(row_o >= off, row_o < off + Dh)
        old = ot_sc[g, pl.ds(w0, _WIN), :]
        ot_sc[g, pl.ds(w0, _WIN), :] = jnp.where(o_in, ot / l, old)

    ot_sc[...] = jnp.zeros_like(ot_sc)
    scores(0, st_a, m_a)

    def pair(i, carry):
        h = 2 * i
        scores(h + 1, st_b, m_b)
        values(h, st_a, m_a)
        scores(jnp.minimum(h + 2, _H - 1), st_a, m_a)
        values(h + 1, st_b, m_b)
        return carry

    jax.lax.fori_loop(0, _H // 2, pair, 0)

    o = jnp.concatenate([ot_sc[g].T.astype(jnp.bfloat16) for g in range(ngrp)], axis=1)
    attn = jnp.dot(o, wo_ref[...], preferred_element_type=jnp.float32)
    h = x_ref[pl.ds(q0, tq), :].astype(jnp.float32) + attn
    hn = _layernorm(h).astype(jnp.bfloat16)

    F = w1_ref.shape[1]
    acc = h
    for c in range(F // fchunk):
        cs = slice(c * fchunk, (c + 1) * fchunk)
        a = jnp.dot(hn, w1_ref[:, cs], preferred_element_type=jnp.float32) + b1_ref[:, cs].astype(jnp.float32)
        t = jnp.exp(-jnp.abs(a))
        pos = a >= 0
        num = jnp.where(pos, 1.0 + 2.0 * t, t * t + 2.0 * t)
        den = jnp.where(pos, num + 2.0 * t * t, num + 2.0)
        act = a * num / den
        acc = acc + jnp.dot(act.astype(jnp.bfloat16), w2_ref[cs, :], preferred_element_type=jnp.float32)
    o_ref[...] = acc.astype(o_ref.dtype)


def _group_cols(w, Dh, hpg, ngrp):
    D = w.shape[0]
    w = w.reshape(D, _H, Dh)
    w = jnp.pad(w, ((0, 0), (0, ngrp * hpg - _H), (0, 0)))
    w = w.reshape(D, ngrp, hpg * Dh)
    w = jnp.pad(w, ((0, 0), (0, 0), (0, _LANES - hpg * Dh)))
    return w.reshape(D, ngrp * _LANES)


@jax.jit
def pallas_sequential_preLN__mha_block__dense_activation_mish__prompt_kernel(
    A_x: jax.Array,
    A_wqkv: jax.Array,
    A_wo: jax.Array,
    B_x: jax.Array,
    B_w1: jax.Array,
    B_b1: jax.Array,
    B_w2: jax.Array,
):
    B, S, D = A_x.shape
    F = B_w1.shape[1]
    Dh = D // _H
    hpg = _LANES // Dh
    ngrp = -(-_H // hpg)
    G = ngrp * _LANES
    tq = 512
    fchunk = 512

    x = A_x.reshape(S, D)
    wq = _group_cols(A_wqkv[:, :D], Dh, hpg, ngrp)
    wk = _group_cols(A_wqkv[:, D:2 * D], Dh, hpg, ngrp)
    wv = _group_cols(A_wqkv[:, 2 * D:], Dh, hpg, ngrp)
    wqv = jnp.concatenate([wq, wv], axis=1)
    wo = _group_cols(A_wo.T, Dh, hpg, ngrp).T
    b1 = B_b1.reshape(1, F)

    full = lambda shape: pl.BlockSpec(shape, lambda i: (0,) * len(shape))
    out = pl.pallas_call(
        functools.partial(_kernel, S=S, D=D, Dh=Dh, hpg=hpg, ngrp=ngrp, tq=tq, fchunk=fchunk),
        grid=(S // tq,),
        in_specs=[full((S, D)), full((D, G)), full((D, 2 * G)), full((G, D)),
                  full((D, F)), full((1, F)), full((F, D))],
        out_specs=pl.BlockSpec((tq, D), lambda i: (i, 0)),
        out_shape=jax.ShapeDtypeStruct((S, D), A_x.dtype),
        scratch_shapes=[
            pltpu.VMEM((ngrp, S, _LANES), jnp.bfloat16),
            pltpu.VMEM((ngrp, _LANES, S), jnp.bfloat16),
            pltpu.VMEM((ngrp, _LANES, S), jnp.bfloat16),
            pltpu.VMEM((ngrp, _LANES, tq), jnp.float32),
            pltpu.VMEM((S, tq), jnp.float32),
            pltpu.VMEM((S, tq), jnp.float32),
            pltpu.VMEM((1, tq), jnp.float32),
            pltpu.VMEM((1, tq), jnp.float32),
        ],
        compiler_params=pltpu.CompilerParams(
            dimension_semantics=("arbitrary",),
            vmem_limit_bytes=100 * 1024 * 1024,
        ),
    )(x, wk, wqv, wo, B_w1, b1, B_w2)
    return out.reshape(B, S, D)
```

```python
import functools
import math

import jax
import jax.numpy as jnp
import jax.experimental.pallas as pl
import jax.experimental.pallas.tpu as pltpu

_H = 32
_LANES = 128
_WIN = 32
_EPS = 1e-5
_LOG2E = math.log2(math.e)


def _layernorm_t(xt):
    m = jnp.mean(xt, axis=0, keepdims=True)
    xc = xt - m
    v = jnp.mean(xc * xc, axis=0, keepdims=True)
    return xc * jax.lax.rsqrt(v + _EPS)


def _kernel(xt_hbm, wqkv_ref, wo_ref, w1_hbm, b1_ref, w2t_hbm, o_ref,
            wg_sc, wqvt_sc, wot_sc, w1_sc, w2t_sc,
            xt_ref, k_sc, qt_sc, vt_sc, ot_sc, st_a, st_b, m_a, m_b, sems,
            *, S, D, Dh, hpg, ngrp, tq, fchunk, pr, ck):
    step = pl.program_id(0)
    G = ngrp * _LANES
    F = w1_sc.shape[1]
    DP = w1_sc.shape[0]

    x_copy = pltpu.make_async_copy(xt_hbm, xt_ref, sems.at[2])
    w1_copy = pltpu.make_async_copy(w1_hbm, w1_sc.at[pl.ds(0, D), :], sems.at[0])
    w2_copy = pltpu.make_async_copy(w2t_hbm, w2t_sc, sems.at[1])

    @pl.when(step == 0)
    def _prologue():
        x_copy.start()
        w1_copy.start()
        w2_copy.start()
        qscale = (Dh ** -0.5) * _LOG2E

        wg_sc[...] = jnp.zeros_like(wg_sc)
        wot_sc[...] = jnp.zeros_like(wot_sc)
        wo_t = wo_ref[...].T
        for g in range(ngrp):
            n = min(hpg, _H - g * hpg) * Dh
            c0 = g * hpg * Dh
            for part in range(3):
                j = part * ngrp + g
                wg_sc[:, j * _LANES:j * _LANES + n] = wqkv_ref[:, part * D + c0:part * D + c0 + n]
            wot_sc[:, g * _LANES:g * _LANES + n] = wo_t[:, c0:c0 + n]
        wqvt_sc[0:G, :] = wg_sc[:, 0:G].T
        wqvt_sc[G:2 * G, :] = wg_sc[:, 2 * G:3 * G].T

        x_copy.wait()

        def cols(r, carry):
            r0 = pl.multiple_of(r * pr, pr)
            xnt = _layernorm_t(xt_ref[:, pl.ds(r0, pr)].astype(jnp.float32)).astype(jnp.bfloat16)
            qvt = jnp.dot(wqvt_sc[...], xnt, preferred_element_type=jnp.float32)
            k = jax.lax.dot_general(xnt, wg_sc[:, G:2 * G], (((0,), (0,)), ((), ())),
                                    preferred_element_type=jnp.float32)
            for g in range(ngrp):
                qt_sc[g, :, pl.ds(r0, pr)] = (qvt[g * _LANES:(g + 1) * _LANES] * qscale).astype(jnp.bfloat16)
                vt_sc[g, :, pl.ds(r0, pr)] = qvt[G + g * _LANES:G + (g + 1) * _LANES].astype(jnp.bfloat16)
                k_sc[g, pl.ds(r0, pr), :] = k[:, g * _LANES:(g + 1) * _LANES].astype(jnp.bfloat16)
            return carry

        jax.lax.fori_loop(0, S // pr, cols, 0)

    q0 = pl.multiple_of(step * tq, tq)
    row_q = jax.lax.broadcasted_iota(jnp.int32, (_LANES, tq), 0)
    row_v = jax.lax.broadcasted_iota(jnp.int32, (_WIN, S), 0)
    row_o = jax.lax.broadcasted_iota(jnp.int32, (_WIN, tq), 0)

    def masked_qt(h, qoff):
        g = h // hpg
        lo = (h % hpg) * Dh
        qt_g = qt_sc[g, :, pl.ds(qoff, tq)]
        in_head = jnp.logical_and(row_q >= lo, row_q < lo + Dh)
        return g, jnp.where(in_head, qt_g, jnp.zeros_like(qt_g))

    def attn_step(h_pv, st_pv, m_pv, h_qk, qoff, st_qk, m_qk):
        gq, qt_h = masked_qt(h_qk, qoff)
        g = h_pv // hpg
        lo = (h_pv % hpg) * Dh
        w0 = pl.multiple_of((lo // 16) * 16, 16)
        off = lo - w0
        v_in = jnp.logical_and(row_v >= off, row_v < off + Dh)
        vwin = vt_sc[g, pl.ds(w0, _WIN), :]
        lhs = jnp.where(v_in, vwin, jnp.ones_like(vwin))
        mcur = m_pv[...]
        mrun = None
        ot = None
        for c in range(S // ck):
            rs = slice(c * ck, (c + 1) * ck)
            st = jnp.dot(k_sc[gq, rs, :], qt_h, preferred_element_type=jnp.float32)
            st_qk[rs, :] = st
            mm = jnp.max(st, axis=0, keepdims=True)
            mrun = mm if mrun is None else jnp.maximum(mrun, mm)
            pt = jnp.exp2(st_pv[rs, :] - mcur).astype(jnp.bfloat16)
            oc = jnp.dot(lhs[:, rs], pt, preferred_element_type=jnp.float32)
            ot = oc if ot is None else ot + oc
        m_qk[...] = mrun
        l = ot[_WIN - 1:_WIN, :]
        o_in = jnp.logical_and(row_o >= off, row_o < off + Dh)
        old = ot_sc[g, pl.ds(w0, _WIN), :]
        ot_sc[g, pl.ds(w0, _WIN), :] = jnp.where(o_in, ot / l, old)

    ot_sc[...] = jnp.zeros_like(ot_sc)

    @pl.when(step == 0)
    def _first_scores():
        g0, qt_0 = masked_qt(0, q0)
        st0 = jnp.dot(k_sc[g0], qt_0, preferred_element_type=jnp.float32)
        st_a[...] = st0
        m_a[...] = jnp.max(st0, axis=0, keepdims=True)

    q_next = pl.multiple_of(jnp.minimum(q0 + tq, S - tq), tq)

    def pair(i, carry):
        h = 2 * i
        attn_step(h, st_a, m_a, h + 1, q0, st_b, m_b)
        last = h + 2 >= _H
        attn_step(h + 1, st_b, m_b, jnp.where(last, 0, h + 2),
                  pl.multiple_of(jnp.where(last, q_next, q0), tq), st_a, m_a)
        return carry

    jax.lax.fori_loop(0, _H // 2, pair, 0)

    @pl.when(step == 0)
    def _ffn_weights():
        w1_copy.wait()
        w2_copy.wait()
        w1_sc[D:DP, :] = jnp.zeros((DP - D, F), jnp.bfloat16)
        w1_sc[D:D + 1, :] = b1_ref[...]

    ot_all = ot_sc[...].reshape(G, tq).astype(jnp.bfloat16)
    attn_t = jnp.dot(wot_sc[...], ot_all, preferred_element_type=jnp.float32)
    ht = xt_ref[:, pl.ds(q0, tq)].astype(jnp.float32) + attn_t
    hnt = _layernorm_t(ht).astype(jnp.bfloat16)
    row_b = jax.lax.broadcasted_iota(jnp.int32, (DP - D, tq), 0)
    hnt = jnp.concatenate([hnt, jnp.where(row_b == 0, 1.0, 0.0).astype(jnp.bfloat16)], axis=0)

    def ffn_chunk(c, acc):
        c0 = pl.multiple_of(c * fchunk, fchunk)
        a = jax.lax.dot_general(w1_sc[:, pl.ds(c0, fchunk)], hnt, (((0,), (0,)), ((), ())),
                                preferred_element_type=jnp.float32)
        t = jnp.exp(-jnp.abs(a))
        pos = a >= 0
        num = jnp.where(pos, 1.0 + 2.0 * t, t * t + 2.0 * t)
        den = jnp.where(pos, num + 2.0 * t * t, num + 2.0)
        act = a * num / den
        return acc + jnp.dot(w2t_sc[:, pl.ds(c0, fchunk)], act.astype(jnp.bfloat16),
                             preferred_element_type=jnp.float32)

    acc = jax.lax.fori_loop(0, F // fchunk, ffn_chunk, ht)
    o_ref[...] = acc.astype(o_ref.dtype)


@jax.jit
def pallas_sequential_preLN__mha_block__dense_activation_mish__prompt_kernel(
    A_x: jax.Array,
    A_wqkv: jax.Array,
    A_wo: jax.Array,
    B_x: jax.Array,
    B_w1: jax.Array,
    B_b1: jax.Array,
    B_w2: jax.Array,
):
    B, S, D = A_x.shape
    F = B_w1.shape[1]
    Dh = D // _H
    hpg = _LANES // Dh
    ngrp = -(-_H // hpg)
    G = ngrp * _LANES
    DP = -(-(D + 1) // _LANES) * _LANES
    tq = 512
    fchunk = F
    pr = 512
    ck = 128

    xt = A_x.reshape(S, D).T
    w2t = B_w2.T
    b1 = B_b1.reshape(1, F)

    full = lambda shape: pl.BlockSpec(shape, lambda i: (0,) * len(shape))
    bf16 = jnp.bfloat16
    out_t = pl.pallas_call(
        functools.partial(_kernel, S=S, D=D, Dh=Dh, hpg=hpg, ngrp=ngrp, tq=tq,
                          fchunk=fchunk, pr=pr, ck=ck),
        grid=(S // tq,),
        in_specs=[pl.BlockSpec(memory_space=pl.ANY), full((D, 3 * D)), full((D, D)),
                  pl.BlockSpec(memory_space=pl.ANY), full((1, F)),
                  pl.BlockSpec(memory_space=pl.ANY)],
        out_specs=pl.BlockSpec((D, tq), lambda i: (0, i)),
        out_shape=jax.ShapeDtypeStruct((D, S), A_x.dtype),
        scratch_shapes=[
            pltpu.VMEM((D, 3 * G), bf16),
            pltpu.VMEM((2 * G, D), bf16),
            pltpu.VMEM((D, G), bf16),
            pltpu.VMEM((DP, F), bf16),
            pltpu.VMEM((D, F), bf16),
            pltpu.VMEM((D, S), bf16),
            pltpu.VMEM((ngrp, S, _LANES), bf16),
            pltpu.VMEM((ngrp, _LANES, S), bf16),
            pltpu.VMEM((ngrp, _LANES, S), bf16),
            pltpu.VMEM((ngrp, _LANES, tq), jnp.float32),
            pltpu.VMEM((S, tq), jnp.float32),
            pltpu.VMEM((S, tq), jnp.float32),
            pltpu.VMEM((1, tq), jnp.float32),
            pltpu.VMEM((1, tq), jnp.float32),
            pltpu.SemaphoreType.DMA((3,)),
        ],
        compiler_params=pltpu.CompilerParams(
            dimension_semantics=("arbitrary",),
            vmem_limit_bytes=110 * 1024 * 1024,
        ),
    )(xt, A_wqkv, A_wo, B_w1, b1, w2t)
    return out_t.T.reshape(B, S, D)
```
